```python
import jax
import jax.numpy as jnp

def _softmax(x, axis=-1):
    return jax.nn.softmax(x, axis=axis)
def _gelu(x):
    return jax.nn.gelu(x, approximate=True)
def _silu(x):
    return jax.nn.silu(x)
def _sigmoid(x):
    return jax.nn.sigmoid(x)
def _layernorm(x, axis=-1, eps=1e-5):
    m = jnp.mean(x, axis=axis, keepdims=True)
    v = jnp.var(x, axis=axis, keepdims=True)
    return (x - m) / jnp.sqrt(v + eps)
def _scatter_add(tgt, idx, src, axis=0):
    return tgt.at[idx].add(src)
def _segment_sum(src, seg, n):
    return jax.ops.segment_sum(src, seg, n)
class _Rng:
    def __init__(self, key):
        self._k = key
    def _next(self):
        self._k, sub = jax.random.split(self._k)
        return sub
    def normal(self, shape):
        return jax.random.normal(self._next(), shape, dtype=jnp.bfloat16)
    def randint(self, lo, hi, shape):
        return jax.random.randint(self._next(), shape, lo, hi, dtype=jnp.int32)
    def uniform(self, shape, lo=0.0, hi=1.0):
        return jax.random.uniform(self._next(), shape, jnp.bfloat16, lo, hi)
    def permutation(self, n):
        return jax.random.permutation(self._next(), n)


kernel_name = 'recurrent_scan__sliding_block_cached__mixer_s_mlp__decode'

def setup_inputs():
    _rng = _Rng(jax.random.key(int.from_bytes(__import__("os").urandom(4), "little")))
    _w = (lambda a: (lambda t: t.astype(jnp.bfloat16) if jnp.issubdtype(t.dtype, jnp.floating) else t)(jnp.asarray(a)))
    def _A_setup():
        B, Sq, D = 1, 1, 512
        Hq, Hkv, Sk, Dh = 32, 32, 32768, 128
        assert Hq % Hkv == 0, (Hq, Hkv)
        return {
            "x": _w((lambda *s: _rng.normal(s) * 0.05)(B, Sq, D)),
            "k_cache": _w((lambda *s: _rng.normal(s) * 0.05)(B, Hkv, Sk, Dh)),
            "v_cache": _w((lambda *s: _rng.normal(s) * 0.05)(B, Hkv, Sk, Dh)),
            "wq": _w((lambda *s: _rng.normal(s) * 0.05)(D, Hq * Dh) * (D ** -0.5)),
            "wo": _w((lambda *s: _rng.normal(s) * 0.05)(Hq * Dh, D) * ((Hq * Dh) ** -0.5)),
        }
    _A_in = _A_setup()

    def _B_setup():
        B, S, D, F = 1, 1, 512, 1376
        return {
            "x":  _w((lambda *s: _rng.normal(s) * 0.05)(B, S, D)),
            "w1": _w((lambda *s: _rng.normal(s) * 0.05)(D, D) * (D ** -0.5)),
            "w2": _w((lambda *s: _rng.normal(s) * 0.05)(D, D) * (D ** -0.5)),
            "w3": _w((lambda *s: _rng.normal(s) * 0.05)(D, F) * (D ** -0.5)),
            "w4": _w((lambda *s: _rng.normal(s) * 0.05)(F, D) * (F ** -0.5)),
        }
    _B_in = _B_setup()

    return {
        "A_x": _A_in["x"],
        "A_k_cache": _A_in["k_cache"],
        "A_v_cache": _A_in["v_cache"],
        "A_wq": _A_in["wq"],
        "A_wo": _A_in["wo"],
        "B_x": _B_in["x"],
        "B_w1": _B_in["w1"],
        "B_w2": _B_in["w2"],
        "B_w3": _B_in["w3"],
        "B_w4": _B_in["w4"],
    }

def reference(A_x, A_k_cache, A_v_cache, A_wq, A_wo, B_x, B_w1, B_w2, B_w3, B_w4):
    def _A_ref(x, k_cache, v_cache, wq, wo):
        B, Sq, D = x.shape
        Hq, Dh = 32, 128
        Hkv, Sk = k_cache.shape[1], k_cache.shape[2]
        W = min(4096, max(256, Sk // 4))
        rep = Hq // Hkv
        q = (lambda x, *d: x.transpose(*d))((x @ wq).reshape(B, Sq, Hq, Dh), 0, 2, 1, 3)
        k = jnp.repeat(k_cache[:, :, Sk - W:, :], rep, axis=1)
        v = jnp.repeat(v_cache[:, :, Sk - W:, :], rep, axis=1)
        scores = jnp.einsum("bhqd,bhkd->bhqk", q, k) * (Dh ** -0.5)
        p = _softmax(scores, axis=-1)
        o = jnp.einsum("bhqk,bhkd->bhqd", p, v)
        return (lambda x, *d: x.transpose(*d))(o, 0, 2, 1, 3).reshape(B, Sq, Hq * Dh) @ wo

    def _B_ref(x, w1, w2, w3, w4):
        B, S, D = x.shape
        h = _gelu(_layernorm(x, axis=-1) @ w1)
        c = D // 4
        g0 = jnp.pad(h[:, :, 0*c:1*c], ((0, 0), (1, 0), (0, 0)))[:, :S, :]
        g1 = jnp.pad(h[:, :, 1*c:2*c], ((0, 0), (0, 1), (0, 0)))[:, 1:, :]
        g2 = jnp.pad(h[:, :, 2*c:3*c], ((0, 0), (2, 0), (0, 0)))[:, :S, :]
        g3 = jnp.pad(h[:, :, 3*c:   ], ((0, 0), (0, 2), (0, 0)))[:, 2:, :]
        hs = jnp.concatenate([g0, g1, g2, g3], axis=-1) @ w2
        x1 = x + hs
        h2 = _gelu(_layernorm(x1, axis=-1) @ w3) @ w4
        return x1 + h2

    x = A_x
    xn = _layernorm(x, axis=-1)
    s = _A_ref(xn, A_k_cache, A_v_cache, A_wq, A_wo)
    g = _silu(_B_ref(xn, B_w1, B_w2, B_w3, B_w4))
    return x + s * g
```

```python
import jax
import jax.numpy as jnp
import numpy as np
import jax.experimental.pallas as pl
import jax.experimental.pallas.tpu as pltpu

HQ, DH = 32, 128
MR = 8
NTAIL = 2
NT = (((1,), (1,)), ((), ()))


def _layernorm(x):
    c = x - jnp.mean(x, axis=-1, keepdims=True)
    v = jnp.mean(c * c, axis=-1, keepdims=True)
    return c / jnp.sqrt(v + 1e-5)


def _gelu(x):
    c = float(np.sqrt(2.0 / np.pi))
    return 0.5 * x * (1.0 + jnp.tanh(c * (x + 0.044715 * (x * x * x))))


@jax.jit
def pallas_recurrent_scan__sliding_block_cached__mixer_s_mlp__decode_kernel(
    A_x: jax.Array,
    A_k_cache: jax.Array,
    A_v_cache: jax.Array,
    A_wq: jax.Array,
    A_wo: jax.Array,
    B_x: jax.Array,
    B_w1: jax.Array,
    B_w2: jax.Array,
    B_w3: jax.Array,
    B_w4: jax.Array,
):
    B, S, D = A_x.shape
    Hkv, Sk = A_k_cache.shape[1], A_k_cache.shape[2]
    assert B == 1 and S == 1 and Hkv == HQ
    W = min(4096, max(256, Sk // 4))
    f32, dt = jnp.float32, A_x.dtype
    nmain = HQ - NTAIL
    split = nmain * DH

    def kernel(x_hbm, k_hbm, v_hbm, wq_hbm, wo_hbm, w3t_hbm, w4_hbm, o_ref,
               x_v, kb, vb, wq_v, wo_v, w3t_v, w4_v, q_s, sem):
        s0, s1 = sem.at[0], sem.at[1]

        def kc(h):
            return pltpu.make_async_copy(k_hbm.at[0, h, pl.ds(Sk - W, W), :], kb.at[h % 2], s1)

        def vc(h):
            return pltpu.make_async_copy(v_hbm.at[0, h, pl.ds(Sk - W, W), :], vb.at[h % 2], s0)

        cx = pltpu.make_async_copy(x_hbm, x_v, s0)
        cq = pltpu.make_async_copy(wq_hbm, wq_v, s1)
        c3 = pltpu.make_async_copy(w3t_hbm, w3t_v, s0)
        c4 = pltpu.make_async_copy(w4_hbm, w4_v, s1)
        head_rows, tail_rows = pl.ds(0, split), pl.ds(split, NTAIL * DH)
        co = pltpu.make_async_copy(wo_hbm.at[head_rows], wo_v.at[head_rows], s0)
        co_tail = pltpu.make_async_copy(wo_hbm.at[tail_rows], wo_v.at[tail_rows], s1)

        cx.start()
        cq.start()
        cx.wait()
        c3.start()
        x = x_v[0].astype(f32)
        xn = jnp.broadcast_to(_layernorm(x).astype(dt), (MR, D))

        cq.wait()
        c4.start()
        q = jnp.dot(xn, wq_v[...], preferred_element_type=f32).astype(dt)
        for h in range(HQ):
            q_s[h] = q[:, h * DH:(h + 1) * DH]

        c3.wait()
        co.start()
        x1 = xn.astype(f32)
        y = _layernorm(x1).astype(dt)
        h2 = _gelu(jax.lax.dot_general(y, w3t_v[...], NT, preferred_element_type=f32)).astype(dt)
        c4.wait()
        kc(0).start()
        b = x1 + jnp.dot(h2, w4_v[...], preferred_element_type=f32)
        g = b * jax.nn.sigmoid(b)
        co.wait()
        vc(0).start()

        def attend(h, next_k, next_v):
            kc(h).wait()
            next_k.start()
            sc = jax.lax.dot_general(q_s[h], kb[h % 2], NT, preferred_element_type=f32) * (DH ** -0.5)
            p = jnp.exp(sc - jnp.max(sc, axis=-1, keepdims=True))
            l = jnp.sum(p, axis=-1, keepdims=True)
            p = p.astype(dt)
            vc(h).wait()
            if next_v is not None:
                next_v.start()
            return (jnp.dot(p, vb[h % 2], preferred_element_type=f32) / l).astype(dt)

        def body(h, acc):
            o = attend(h, kc(h + 1), vc(h + 1))
            wo_h = wo_v[pl.ds(pl.multiple_of(h * DH, DH), DH), :]
            return acc + jnp.dot(o, wo_h, preferred_element_type=f32)

        acc = jax.lax.fori_loop(0, nmain, body, jnp.zeros((MR, D), f32))

        tail = [attend(h, kc(h + 1), vc(h + 1)) for h in range(nmain, HQ - 1)]
        tail.append(attend(HQ - 1, co_tail, None))
        o_tail = jnp.concatenate(tail, axis=1)
        co_tail.wait()
        acc = acc + jnp.dot(o_tail, wo_v[split:, :], preferred_element_type=f32)
        o_ref[0] = (x + acc[0:1] * g[0:1]).astype(o_ref.dtype)

    w3t = B_w3.T
    return pl.pallas_call(
        kernel,
        out_shape=jax.ShapeDtypeStruct(A_x.shape, dt),
        in_specs=[pl.BlockSpec(memory_space=pl.ANY)] * 7,
        out_specs=pl.BlockSpec(memory_space=pltpu.VMEM),
        scratch_shapes=[
            pltpu.VMEM(A_x.shape, dt),
            pltpu.VMEM((2, W, DH), A_k_cache.dtype),
            pltpu.VMEM((2, W, DH), A_v_cache.dtype),
            pltpu.VMEM(A_wq.shape, A_wq.dtype),
            pltpu.VMEM(A_wo.shape, A_wo.dtype),
            pltpu.VMEM(w3t.shape, w3t.dtype),
            pltpu.VMEM(B_w4.shape, B_w4.dtype),
            pltpu.VMEM((HQ, MR, DH), dt),
            pltpu.SemaphoreType.DMA((2,)),
        ],
        compiler_params=pltpu.CompilerParams(vmem_limit_bytes=32 * 1024 * 1024),
    )(A_x, A_k_cache, A_v_cache, A_wq, A_wo, w3t, B_w4)
```
